```python
import jax
import jax.numpy as jnp

def _softmax(x, axis=-1):
    return jax.nn.softmax(x, axis=axis)
def _gelu(x):
    return jax.nn.gelu(x, approximate=True)
def _silu(x):
    return jax.nn.silu(x)
def _sigmoid(x):
    return jax.nn.sigmoid(x)
def _layernorm(x, axis=-1, eps=1e-5):
    m = jnp.mean(x, axis=axis, keepdims=True)
    v = jnp.var(x, axis=axis, keepdims=True)
    return (x - m) / jnp.sqrt(v + eps)
def _scatter_add(tgt, idx, src, axis=0):
    return tgt.at[idx].add(src)
def _segment_sum(src, seg, n):
    return jax.ops.segment_sum(src, seg, n)
class _Rng:
    def __init__(self, key):
        self._k = key
    def _next(self):
        self._k, sub = jax.random.split(self._k)
        return sub
    def normal(self, shape):
        return jax.random.normal(self._next(), shape, dtype=jnp.bfloat16)
    def randint(self, lo, hi, shape):
        return jax.random.randint(self._next(), shape, lo, hi, dtype=jnp.int32)
    def uniform(self, shape, lo=0.0, hi=1.0):
        return jax.random.uniform(self._next(), shape, jnp.bfloat16, lo, hi)
    def permutation(self, n):
        return jax.random.permutation(self._next(), n)


kernel_name = 'concat_heads__mha_block_cached__compressed_kv_cla__decode'

def setup_inputs():
    _rng = _Rng(jax.random.key(int.from_bytes(__import__("os").urandom(4), "little")))
    _w = (lambda a: (lambda t: t.astype(jnp.bfloat16) if jnp.issubdtype(t.dtype, jnp.floating) else t)(jnp.asarray(a)))
    def _A_setup():
        B, Sq, D = 4, 1, 576
        H, Sk, Dh = 32, 4096, 128
        return {
            "x": _w((lambda *s: _rng.normal(s) * 0.05)(B, Sq, D)),
            "k_cache": _w((lambda *s: _rng.normal(s) * 0.05)(B, H, Sk, Dh)),
            "v_cache": _w((lambda *s: _rng.normal(s) * 0.05)(B, H, Sk, Dh)),
            "wq": _w((lambda *s: _rng.normal(s) * 0.05)(D, H * Dh) * (D ** -0.5)),
            "wo": _w((lambda *s: _rng.normal(s) * 0.05)(H * Dh, D) * ((H * Dh) ** -0.5)),
        }
    _A_in = _A_setup()

    def _B_setup():
        B, H, Sq, Sk, D, M = 4, 32, 1, 4096, 128, 576
        Dc = 4 * D
        return {
            "x": _w((lambda *s: _rng.normal(s) * 0.05)(B, Sq, M)),
            "c_kv": _w((lambda *s: _rng.normal(s) * 0.05)(B, Sk, Dc)),
            "w_q": _w((lambda *s: _rng.normal(s) * 0.05)(M, H, D) * (M ** -0.5)),
            "w_uk": _w((lambda *s: _rng.normal(s) * 0.05)(Dc, H, D) * (Dc ** -0.5)),
            "w_uv": _w((lambda *s: _rng.normal(s) * 0.05)(Dc, H, D) * (Dc ** -0.5)),
            "w_o": _w((lambda *s: _rng.normal(s) * 0.05)(H, D, M) * ((H * D) ** -0.5)),
        }
    _B_in = _B_setup()

    return {
        "A_x": _A_in["x"],
        "A_k_cache": _A_in["k_cache"],
        "A_v_cache": _A_in["v_cache"],
        "A_wq": _A_in["wq"],
        "A_wo": _A_in["wo"],
        "B_x": _B_in["x"],
        "B_c_kv": _B_in["c_kv"],
        "B_w_q": _B_in["w_q"],
        "B_w_uk": _B_in["w_uk"],
        "B_w_uv": _B_in["w_uv"],
        "B_w_o": _B_in["w_o"],
    }

def reference(A_x, A_k_cache, A_v_cache, A_wq, A_wo, B_x, B_c_kv, B_w_q, B_w_uk, B_w_uv, B_w_o):
    def _A_ref(x, k_cache, v_cache, wq, wo):
        B, Sq, D = x.shape
        H, Dh = 32, 128
        q = (lambda x, *d: x.transpose(*d))((x @ wq).reshape(B, Sq, H, Dh), 0, 2, 1, 3)
        scores = jnp.einsum("bhqd,bhkd->bhqk", q, k_cache) * (Dh ** -0.5)
        p = _softmax(scores, axis=-1)
        o = jnp.einsum("bhqk,bhkd->bhqd", p, v_cache)
        return (lambda x, *d: x.transpose(*d))(o, 0, 2, 1, 3).reshape(B, Sq, H * Dh) @ wo

    def _B_ref(x, c_kv, w_q, w_uk, w_uv, w_o):
        B, Sq, M = x.shape[0], x.shape[1], x.shape[2]
        Sk = c_kv.shape[1]
        H, D = w_q.shape[1], w_q.shape[2]
        q = jnp.einsum("bqm,mhd->bhqd", x, w_q)
        k = jnp.einsum("bkc,chd->bhkd", c_kv, w_uk)
        v = jnp.einsum("bkc,chd->bhkd", c_kv, w_uv)
        scores = jnp.einsum("bhqd,bhkd->bhqk", q, k) * (D ** -0.5)
        off = Sk - Sq
        qi = jnp.arange(Sq)[:, None]
        kj = jnp.arange(Sk)[None, :]
        cmask = kj <= (qi + off)
        scores = jnp.where(cmask[None, None], scores, -1e9)
        p = _softmax(scores, axis=-1)
        ctx = jnp.einsum("bhqk,bhkd->bhqd", p, v)
        return jnp.einsum("bhqd,hdm->bqm", ctx, w_o)

    a = _A_ref(A_x, A_k_cache, A_v_cache, A_wq, A_wo)
    b = _B_ref(B_x, B_c_kv, B_w_q, B_w_uk, B_w_uv, B_w_o)
    return jnp.concatenate([a, b], axis=-1)
```

```python
import functools

import jax
import jax.numpy as jnp
from jax import lax
import jax.experimental.pallas as pl
import jax.experimental.pallas.tpu as pltpu

BF16 = jnp.bfloat16
F32 = jnp.float32

NB, NH, SK, DH, DM, DC = 4, 32, 4096, 128, 576, 512
HG = 8
NG = NB * NH // HG
GPB = NH // HG


def _nt(a, b):
    return lax.dot_general(a, b, (((1,), (1,)), ((), ())), preferred_element_type=F32)


def _nn(a, b):
    return jnp.dot(a, b, preferred_element_type=F32)


def _iota(shape, dim):
    return lax.broadcasted_iota(jnp.int32, shape, dim)


def _loop(lo, hi, fn):
    def body(t, c):
        fn(t)
        return c
    lax.fori_loop(lo, hi, body, 0)


def make(run=256, look=5, nslot=8, nochk=False, compute=True):
    R = SK // run
    NKV = NG * R
    NC = 16
    NO = 8
    scale = DH ** -0.5

    def kernel(xa_h, k_h, v_h, wq_h, wo_h, xb_h, c_h, bq_h, uk_h, uv_h, bo_h, out_ref,
               xa_v, xb_v, wq_v, bq_v, uk_v, uv_v, c_v, kv_v, wo_v, bo_v,
               bqt_v, qa_v, qb_v, lat_v, ql_v, mb_v, lb_v, ab_v, oa_v, ob_v,
               sem_w, sem_c, sem_kv, sem_o):

        def start(src, dst, sem, q):
            pltpu.make_async_copy(src, dst, sem).start(priority=q)

        def wait(dst, sem):
            pltpu.make_async_copy(dst, dst, sem).wait()

        def issue_w1(t):
            for s in range(4):
                rows = pl.ds(pl.multiple_of((s * 9 + t // 4) * 16, 16), 16)
                cb = t % 4
                start(wq_h.at[rows, pl.ds(pl.multiple_of(cb * 1024, 1024), 1024)],
                      wq_v.at[cb, rows], sem_w.at[0], 0)
                idx = (pl.ds((s % 2) * 2, 2), pl.ds((s // 2) * 72 + 2 * t, 2))
                start(bq_h.at[idx], bq_v.at[idx], sem_w.at[1], 1)

        def issue_w2(t):
            for s in range(4):
                idx = (pl.ds((s % 2) * 2, 2), pl.ds((s // 2) * 64 + 2 * t, 2))
                start(uk_h.at[idx], uk_v.at[idx], sem_w.at[2], 0)
                start(uv_h.at[idx], uv_v.at[idx], sem_w.at[3], 1)

        def issue_c(i):
            def rnd(d):
                for s in range(4):
                    for a in range(2):
                        parts = pl.ds(a * 8 + s * 2, 2)
                        start(c_h.at[parts, pl.ds(pl.multiple_of(i * 64 + d * 16, 16), 16)],
                              c_v.at[i, parts, pl.ds(pl.multiple_of(d * 16, 16), 16)],
                              sem_c.at[i], a)
            _loop(0, 4, rnd)

        def issue_kv(i):
            g = i // R
            r = i % R
            u = i % nslot

            def rnd(d):
                for s in range(4):
                    for a, src in enumerate((k_h, v_h)):
                        heads = pl.ds(s * 2, 2)
                        start(src.at[g, heads, pl.ds(pl.multiple_of(r * run + d * 64, 64), 64)],
                              kv_v.at[u, a, heads, pl.ds(pl.multiple_of(d * 64, 64), 64)],
                              sem_kv.at[u], a)
            _loop(0, run // 64, rnd)

        def issue_o(i):
            def rnd(d):
                for s in range(2):
                    rows = pl.ds(pl.multiple_of((s * 9 + d) * 32, 32), 32)
                    start(wo_h.at[rows, pl.ds(pl.multiple_of(i * 512, 512), 512)],
                          wo_v.at[i, rows], sem_o.at[i], 0)
                    rows = pl.ds(pl.multiple_of(d * 64, 64), 64)
                    start(bo_h.at[pl.ds(s * 2, 2), i, rows], bo_v.at[i, pl.ds(s * 2, 2), rows],
                          sem_o.at[i], 1)
            _loop(0, 9, rnd)

        _loop(0, 1, issue_w1)
        start(xa_h, xa_v, sem_w.at[4], 0)
        start(xb_h, xb_v, sem_w.at[5], 1)
        _loop(1, 36, issue_w1)
        _loop(0, 12, issue_w2)
        wait(xa_v, sem_w.at[4])
        wait(xb_v, sem_w.at[5])
        wait(wq_v, sem_w.at[0])
        wait(bq_v, sem_w.at[1])

        xa = xa_v[...].astype(F32)
        xa32 = jnp.concatenate(
            [jnp.broadcast_to(xa[b:b + 1], (HG, DM)) for b in range(NB)], axis=0).astype(BF16)
        xb = xb_v[...].astype(F32)
        xb8 = jnp.concatenate([xb, jnp.zeros_like(xb)], axis=0).astype(BF16)

        def stage1(c):
            if compute:
                bqt_v[:, pl.ds(pl.multiple_of(c * 144, 16), 144), :] = jnp.swapaxes(bq_v[c], 0, 1)
                q = _nn(xa32, wq_v[c])
                diag = (_iota(q.shape, 0) % HG) == (_iota(q.shape, 1) // DH)
                qa_v[c] = jnp.where(diag, q, 0.0)
            _loop(12 + 5 * c, 17 + 5 * c, issue_w2)
        _loop(0, 4, stage1)

        def stage2(c):
            if compute:
                for j in range(8):
                    qb_v[c * 8 + j] = _nn(xb8, bqt_v[c * 8 + j])

            @pl.when(c < look - 2)
            def _():
                issue_c(c)
        _loop(0, 4, stage2)
        wait(uk_v, sem_w.at[2])
        wait(uv_v, sem_w.at[3])

        def stage3(c):
            if compute:
                wt = jnp.swapaxes(uk_v[c], 0, 1)
                ql = jnp.concatenate(
                    [_nt(qb_v[h].astype(BF16), wt[h]) for h in range(NH)], axis=0).astype(BF16)
                row = _iota((NB * NH, NH * 8), 0)
                col = _iota((NB * NH, NH * 8), 1)
                perm = jnp.where(col == (row % NH) * 8 + row // NH, 1.0, 0.0).astype(BF16)
                ql_v[c] = _nn(perm, ql).astype(BF16)

            @pl.when(c % 2 == 1)
            def _():
                issue_c(look - 2 + c // 2)
        _loop(0, 4, stage3)

        mb_v[...] = jnp.full(mb_v.shape, -jnp.inf, F32)
        lb_v[...] = jnp.zeros(lb_v.shape, F32)
        ab_v[...] = jnp.zeros(ab_v.shape, F32)
        oa_v[...] = jnp.zeros(oa_v.shape, F32)
        ob_v[...] = jnp.zeros(ob_v.shape, F32)

        def flash_b(i):
            wait(c_v.at[i], sem_c.at[i])
            if compute:
                for b in range(NB):
                    rows = pl.ds(b * NH, NH)
                    c = c_v[i, pl.ds(4 * b, 4)].reshape(256, DC)
                    q = jnp.concatenate([ql_v[j, rows] for j in range(4)], axis=1)
                    s = _nt(q, c) * scale
                    m_old = mb_v[rows]
                    m_new = jnp.maximum(m_old, jnp.max(s, axis=1, keepdims=True))
                    alpha = jnp.exp(m_old - m_new)
                    p = jnp.exp(s - jnp.tile(m_new, (1, 2)))
                    mb_v[rows] = m_new
                    lb_v[rows] = lb_v[rows] * alpha + (p[:, :128] + p[:, 128:])
                    ab_v[rows] = ab_v[rows] * jnp.tile(alpha, (1, 4)) + _nn(p.astype(BF16), c)

            @pl.when(i + look < NC)
            def _():
                issue_c(i + look)

            @pl.when(i + look >= NC)
            def _():
                issue_kv(i + look - NC)
        _loop(0, NC, flash_b)

        if compute:
            lat = (ab_v[...] / jnp.sum(lb_v[...], axis=1, keepdims=True)).astype(BF16)
            row = _iota((NH * 8, NB * NH), 0)
            col = _iota((NH * 8, NB * NH), 1)
            perm = jnp.where(row == (col % NH) * 8 + col // NH, 1.0, 0.0).astype(BF16)
            lat = _nn(perm, lat)
            for j in range(4):
                lat_v[j] = lat[:, j * 128:(j + 1) * 128]

        sub = _iota((HG, DH), 0)

        def flash_a(i, carry):
            m_old, l_old, acc = carry
            g = i // R
            r = i % R
            u = i % nslot
            b = g // GPB
            hg = g % GPB
            wait(kv_v.at[u], sem_kv.at[u])
            if compute:
                q = qa_v[hg, pl.ds(pl.multiple_of(b * HG, HG), HG), :].astype(BF16)
                s = None
                for j in range(HG):
                    sj = _nt(q[:, j * DH:(j + 1) * DH], kv_v[u, 0, j])
                    s = sj if s is None else s + sj
                s = s * scale
                first = r == 0
                m_old = jnp.where(first, -jnp.inf, m_old)
                m_new = jnp.maximum(m_old, jnp.max(s, axis=1, keepdims=True))
                alpha = jnp.exp(m_old - m_new)
                p = jnp.exp(s - jnp.tile(m_new, (1, run // 128)))
                psum = p[:, :128]
                for t in range(1, run // 128):
                    psum = psum + p[:, t * 128:(t + 1) * 128]
                l_new = jnp.where(first, 0.0, l_old) * alpha + psum
                pb = p.astype(BF16)
                pv = _nn(pb, kv_v[u, 1, 0])
                for j in range(1, HG):
                    pv = jnp.where(sub == j, _nn(pb, kv_v[u, 1, j]), pv)
                acc = jnp.where(first, 0.0, acc) * alpha + pv

                @pl.when(r == R - 1)
                def _():
                    o = acc / jnp.sum(l_new, axis=1, keepdims=True)
                    for j in range(HG):
                        dst = (hg * 2 + j // 4, slice(None), pl.ds((j % 4) * DH, DH))
                        oa_v[dst] = jnp.where(
                            sub == b, jnp.broadcast_to(o[j:j + 1], (HG, DH)), oa_v[dst])

                @pl.when(i < 4)
                def _():
                    wt = jnp.swapaxes(uv_v[i], 0, 1)
                    for h in range(NH):
                        ob_v[h] += _nn(lat_v[i, pl.ds(h * 8, 8)].astype(BF16), wt[h])
            else:
                m_new, l_new = m_old, l_old

            @pl.when(i + look < NKV)
            def _():
                issue_kv(i + look)

            @pl.when(i + look >= NKV)
            def _():
                issue_o(i + look - NKV)
            return m_new, l_new, acc

        z = jnp.zeros((HG, DH), F32)
        lax.fori_loop(0, NKV, flash_a, (z, z, z))

        def proj(i, carry):
            ya, yb = carry
            wait(wo_v.at[i], sem_o.at[i])
            wait(bo_v.at[i], sem_o.at[i])
            if compute:
                ya = ya + _nt(oa_v[i].astype(BF16), wo_v[i])
                for j in range(4):
                    yb = yb + _nt(ob_v[j * 8 + i].astype(BF16), bo_v[i, j])

            @pl.when(i + look < NO)
            def _():
                issue_o(i + look)
            return ya, yb

        z = jnp.zeros((8, DM), F32)
        ya, yb = lax.fori_loop(0, NO, proj, (z, z))
        out_ref[...] = jnp.concatenate([ya[:NB], yb[:NB]], axis=1).astype(BF16)

    def f(A_x, A_k_cache, A_v_cache, A_wq, A_wo, B_x, B_c_kv, B_w_q, B_w_uk, B_w_uv, B_w_o):
        args = (
            A_x.reshape(NB, DM),
            A_k_cache.reshape(NG, HG, SK, DH),
            A_v_cache.reshape(NG, HG, SK, DH),
            A_wq,
            A_wo.T,
            B_x.reshape(NB, DM),
            B_c_kv.reshape(16, 1024, DC),
            B_w_q.reshape(4, 144, NH, DH),
            B_w_uk.reshape(4, 128, NH, DH),
            B_w_uv.reshape(4, 128, NH, DH),
            B_w_o.transpose(0, 2, 1).reshape(4, 8, DM, DH),
        )
        out = pl.pallas_call(
            kernel,
            out_shape=jax.ShapeDtypeStruct((NB, 2 * DM), BF16),
            in_specs=[pl.BlockSpec(memory_space=pl.ANY)] * len(args),
            scratch_shapes=[
                pltpu.VMEM((NB, DM), BF16),
                pltpu.VMEM((NB, DM), BF16),
                pltpu.VMEM((4, DM, 1024), BF16),
                pltpu.VMEM((4, 144, NH, DH), BF16),
                pltpu.VMEM((4, 128, NH, DH), BF16),
                pltpu.VMEM((4, 128, NH, DH), BF16),
                pltpu.VMEM((NC, 16, 64, DC), BF16),
                pltpu.VMEM((nslot, 2, HG, run, DH), BF16),
                pltpu.VMEM((NO, DM, 512), BF16),
                pltpu.VMEM((NO, 4, DM, DH), BF16),
                pltpu.VMEM((NH, DM, DH), BF16),
                pltpu.VMEM((GPB, NB * HG, HG * DH), F32),
                pltpu.VMEM((NH, 8, DH), F32),
                pltpu.VMEM((4, NH * 8, 128), F32),
                pltpu.VMEM((4, NB * NH, 128), BF16),
                pltpu.VMEM((NB * NH, 128), F32),
                pltpu.VMEM((NB * NH, 128), F32),
                pltpu.VMEM((NB * NH, DC), F32),
                pltpu.VMEM((NO, 8, 512), F32),
                pltpu.VMEM((NH, 8, DH), F32),
                pltpu.SemaphoreType.DMA((6,)),
                pltpu.SemaphoreType.DMA((NC,)),
                pltpu.SemaphoreType.DMA((nslot,)),
                pltpu.SemaphoreType.DMA((NO,)),
            ],
            compiler_params=pltpu.CompilerParams(
                vmem_limit_bytes=100 * 1024 * 1024, disable_bounds_checks=nochk),
            name="fused_decode",
        )(*args)
        return out.reshape(NB, 1, 2 * DM)
    return f


@jax.jit
def pallas_concat_heads__mha_block_cached__compressed_kv_cla__decode_kernel(
    A_x, A_k_cache, A_v_cache, A_wq, A_wo, B_x, B_c_kv, B_w_q, B_w_uk, B_w_uv, B_w_o,
):
    return make()(A_x, A_k_cache, A_v_cache, A_wq, A_wo, B_x, B_c_kv, B_w_q, B_w_uk, B_w_uv, B_w_o)
```

```python
import functools

import jax
import jax.numpy as jnp
from jax import lax
import jax.experimental.pallas as pl
import jax.experimental.pallas.tpu as pltpu

BF16 = jnp.bfloat16
F32 = jnp.float32

NB, NH, SK, DH, DM, DC = 4, 32, 4096, 128, 576, 512
HG = 8
NG = NB * NH // HG
GPB = NH // HG


def _nt(a, b):
    return lax.dot_general(a, b, (((1,), (1,)), ((), ())), preferred_element_type=F32)


def _nn(a, b):
    return jnp.dot(a, b, preferred_element_type=F32)


def _iota(shape, dim):
    return lax.broadcasted_iota(jnp.int32, shape, dim)


def _loop(lo, hi, fn):
    def body(t, c):
        fn(t)
        return c
    lax.fori_loop(lo, hi, body, 0)


def make(run=256, look=4, nslot=4, nochk=True, compute='xap', mix=False, skip=''):
    R = SK // run
    NKV = NG * R
    NO = 8
    scale = DH ** -0.5

    def kernel(xa_h, k_h, v_h, wq_h, wo_h, xb_h, c_h, bq_h, uk_h, uv_h, bo_h, out_ref,
               xa_v, xb_v, wq_v, bq_v, uk_v, uv_v, c_v, kv_v, wo_v, bo_v,
               bqt_v, qa_v, qb_v, lat_v, ql_v, mb_v, lb_v, ab_v, oa_v, ob_v,
               sem_w, sem_kv, sem_o):

        def start(src, dst, sem, q):
            pltpu.make_async_copy(src, dst, sem).start(priority=q)

        def wait(dst, sem):
            pltpu.make_async_copy(dst, dst, sem).wait()

        def issue_w1(t):
            if '1' in skip:
                return
            for s in range(4):
                rows = pl.ds(pl.multiple_of((s * 9 + t // 4) * 16, 16), 16)
                cb = t % 4
                start(wq_h.at[rows, pl.ds(pl.multiple_of(cb * 1024, 1024), 1024)],
                      wq_v.at[cb, rows], sem_w.at[0], 0)
                idx = (pl.ds((s % 2) * 2, 2), pl.ds((s // 2) * 72 + 2 * t, 2))
                start(bq_h.at[idx], bq_v.at[idx], sem_w.at[1], 1)

        def issue_w2(t):
            if '2' in skip:
                return
            for s in range(4):
                idx = (pl.ds((s % 2) * 2, 2), pl.ds((s // 2) * 64 + 2 * t, 2))
                start(uk_h.at[idx], uk_v.at[idx], sem_w.at[2], 0)
                start(uv_h.at[idx], uv_v.at[idx], sem_w.at[3], 1)

        def issue_c(t):
            if 'c' in skip:
                return
            for s in range(4):
                for a in range(2):
                    idx = (pl.ds(a * 8 + s * 2, 2), pl.ds(pl.multiple_of(t * 16, 16), 16))
                    start(c_h.at[idx], c_v.at[idx], sem_w.at[6], a)

        def issue_kv(i):
            g = i // R
            r = i % R
            u = i % nslot

            def rnd(d):
                for s in range(4):
                    for a, src in enumerate((k_h, v_h)):
                        heads = pl.ds(s * 2, 2)
                        start(src.at[g, heads, pl.ds(pl.multiple_of(r * run + d * 64, 64), 64)],
                              kv_v.at[u, a, heads, pl.ds(pl.multiple_of(d * 64, 64), 64)],
                              sem_kv.at[u], a)
            _loop(0, run // 64, rnd)

        def issue_o(i):
            if 'o' in skip:
                return

            def rnd(d):
                for s in range(2):
                    rows = pl.ds(pl.multiple_of((s * 9 + d) * 32, 32), 32)
                    start(wo_h.at[rows, pl.ds(pl.multiple_of(i * 512, 512), 512)],
                          wo_v.at[i, rows], sem_o.at[i], 0)
                    rows = pl.ds(pl.multiple_of(d * 64, 64), 64)
                    start(bo_h.at[pl.ds(s * 2, 2), i, rows], bo_v.at[i, pl.ds(s * 2, 2), rows],
                          sem_o.at[i], 1)
            _loop(0, 9, rnd)

        _loop(0, 36, issue_w1)
        start(xa_h, xa_v, sem_w.at[4], 0)
        start(xb_h, xb_v, sem_w.at[5], 1)
        if not mix:
            _loop(0, 32, issue_w2)
            _loop(0, 64, issue_c)
        _loop(0, look - 1, issue_kv)
        wait(xa_v, sem_w.at[4])
        wait(xb_v, sem_w.at[5])
        if '1' not in skip:
            wait(wq_v, sem_w.at[0])
            wait(bq_v, sem_w.at[1])

        mb_v[...] = jnp.full(mb_v.shape, -jnp.inf, F32)
        lb_v[...] = jnp.zeros(lb_v.shape, F32)
        ab_v[...] = jnp.zeros(ab_v.shape, F32)
        oa_v[...] = jnp.zeros(oa_v.shape, F32)
        ob_v[...] = jnp.zeros(ob_v.shape, F32)

        def q_a(c):
            xa = xa_v[...].astype(F32)
            xa32 = jnp.concatenate(
                [jnp.broadcast_to(xa[b:b + 1], (HG, DM)) for b in range(NB)], axis=0)
            q = _nn(xa32.astype(BF16), wq_v[c])
            diag = (_iota(q.shape, 0) % HG) == (_iota(q.shape, 1) // DH)
            qa_v[c] = jnp.where(diag, q, 0.0)

        def bq_t(c):
            bqt_v[:, pl.ds(pl.multiple_of(c * 48, 16), 48), :] = jnp.swapaxes(
                bq_v[c // 3, pl.ds((c % 3) * 48, 48)], 0, 1)

        def q_b(c):
            xb = xb_v[...].astype(F32)
            xb8 = jnp.concatenate([xb, jnp.zeros_like(xb)], axis=0).astype(BF16)
            for j in range(4):
                qb_v[c * 4 + j] = _nn(xb8, bqt_v[c * 4 + j])

        def wait_b(c):
            if '2' not in skip:
                wait(uk_v, sem_w.at[2])
                wait(uv_v, sem_w.at[3])
            if 'c' not in skip:
                wait(c_v, sem_w.at[6])

        def q_lat(c):
            wt = jnp.swapaxes(uk_v[c], 0, 1)
            ql = jnp.concatenate(
                [_nt(qb_v[h].astype(BF16), wt[h]) for h in range(NH)], axis=0).astype(BF16)
            row = _iota((NB * NH, NH * 8), 0)
            col = _iota((NB * NH, NH * 8), 1)
            perm = jnp.where(col == (row % NH) * 8 + row // NH, 1.0, 0.0).astype(BF16)
            ql_v[c] = _nn(perm, ql).astype(BF16)

        def flash_b(t):
            rows = pl.ds(pl.multiple_of((t // 8) * NH, NH), NH)
            c = c_v[t // 2, pl.ds(pl.multiple_of((t % 2) * 512, 512), 512)]
            q = jnp.concatenate([ql_v[j, rows] for j in range(4)], axis=1)
            s = _nt(q, c) * scale
            m_old = mb_v[rows]
            m_new = jnp.maximum(m_old, jnp.max(s, axis=1, keepdims=True))
            alpha = jnp.exp(m_old - m_new)
            p = jnp.exp(s - jnp.tile(m_new, (1, 4)))
            mb_v[rows] = m_new
            lb_v[rows] = lb_v[rows] * alpha + (
                (p[:, :128] + p[:, 128:256]) + (p[:, 256:384] + p[:, 384:]))
            ab_v[rows] = ab_v[rows] * jnp.tile(alpha, (1, 4)) + _nn(p.astype(BF16), c)

        def latent(c):
            lat = (ab_v[...] / jnp.sum(lb_v[...], axis=1, keepdims=True)).astype(BF16)
            row = _iota((NH * 8, NB * NH), 0)
            col = _iota((NH * 8, NB * NH), 1)
            perm = jnp.where(row == (col % NH) * 8 + col // NH, 1.0, 0.0).astype(BF16)
            lat = _nn(perm, lat)
            for j in range(4):
                lat_v[j] = lat[:, j * 128:(j + 1) * 128]

        def ctx_b(c):
            wt = jnp.swapaxes(uv_v[c], 0, 1)
            for h in range(NH):
                ob_v[h] += _nn(lat_v[c, pl.ds(h * 8, 8)].astype(BF16), wt[h])

        side = [(q_a, 4), (bq_t, 12), (q_b, 8), (None, 30), (wait_b, 1), (q_lat, 4),
                (flash_b, 32), (latent, 1), (ctx_b, 4)]

        sub = _iota((HG, DH), 0)

        def flash_a(i, carry):
            m_old, l_old, acc = carry
            g = i // R
            r = i % R
            u = i % nslot
            b = g // GPB
            hg = g % GPB

            @pl.when(i % 2 == 0)
            def _():
                t = i // 2
                lo = 0
                for fn, n in side:
                    if fn is not None and ('x' in compute or fn is wait_b):
                        pl.when((t >= lo) & (t < lo + n))(functools.partial(fn, t - lo))
                    lo += n

            @pl.when(i + look - 1 < NKV)
            def _():
                issue_kv(i + look - 1)

            @pl.when(i + look - 1 >= NKV)
            def _():
                issue_o(i + look - 1 - NKV)

            if mix:
                pl.when(i < 32)(functools.partial(issue_w2, i))
                pl.when((i >= 32) & (i < 96))(functools.partial(issue_c, i - 32))

            wait(kv_v.at[u], sem_kv.at[u])
            if 'a' in compute:
                q = qa_v[hg, pl.ds(pl.multiple_of(b * HG, HG), HG), :].astype(BF16)
                s = None
                for j in range(HG):
                    sj = _nt(q[:, j * DH:(j + 1) * DH], kv_v[u, 0, j])
                    s = sj if s is None else s + sj
                s = s * scale
                first = r == 0
                m_old = jnp.where(first, -jnp.inf, m_old)
                m_new = jnp.maximum(m_old, jnp.max(s, axis=1, keepdims=True))
                alpha = jnp.exp(m_old - m_new)
                p = jnp.exp(s - jnp.tile(m_new, (1, run // 128)))
                psum = p[:, :128]
                for t in range(1, run // 128):
                    psum = psum + p[:, t * 128:(t + 1) * 128]
                l_new = jnp.where(first, 0.0, l_old) * alpha + psum
                pb = p.astype(BF16)
                pv = _nn(pb, kv_v[u, 1, 0])
                for j in range(1, HG):
                    pv = jnp.where(sub == j, _nn(pb, kv_v[u, 1, j]), pv)
                acc = jnp.where(first, 0.0, acc) * alpha + pv

                @pl.when(r == R - 1)
                def _():
                    o = acc / jnp.sum(l_new, axis=1, keepdims=True)
                    for j in range(HG):
                        dst = (hg * 2 + j // 4, slice(None), pl.ds((j % 4) * DH, DH))
                        oa_v[dst] = jnp.where(
                            sub == b, jnp.broadcast_to(o[j:j + 1], (HG, DH)), oa_v[dst])
            else:
                m_new, l_new = m_old, l_old
            return m_new, l_new, acc

        z = jnp.zeros((HG, DH), F32)
        lax.fori_loop(0, NKV, flash_a, (z, z, z))

        def proj(i, carry):
            ya, yb = carry

            @pl.when(i + look - 1 < NO)
            def _():
                issue_o(i + look - 1)
            if 'o' not in skip:
                wait(wo_v.at[i], sem_o.at[i])
                wait(bo_v.at[i], sem_o.at[i])
            if 'p' in compute:
                ya = ya + _nt(oa_v[i].astype(BF16), wo_v[i])
                for j in range(4):
                    yb = yb + _nt(ob_v[j * 8 + i].astype(BF16), bo_v[i, j])
            return ya, yb

        z = jnp.zeros((8, DM), F32)
        ya, yb = lax.fori_loop(0, NO, proj, (z, z))
        out_ref[...] = jnp.concatenate([ya[:NB], yb[:NB]], axis=1).astype(BF16)

    def f(A_x, A_k_cache, A_v_cache, A_wq, A_wo, B_x, B_c_kv, B_w_q, B_w_uk, B_w_uv, B_w_o):
        args = (
            A_x.reshape(NB, DM),
            A_k_cache.reshape(NG, HG, SK, DH),
            A_v_cache.reshape(NG, HG, SK, DH),
            A_wq,
            A_wo.T,
            B_x.reshape(NB, DM),
            B_c_kv.reshape(16, 1024, DC),
            B_w_q.reshape(4, 144, NH, DH),
            B_w_uk.reshape(4, 128, NH, DH),
            B_w_uv.reshape(4, 128, NH, DH),
            B_w_o.transpose(0, 2, 1).reshape(4, 8, DM, DH),
        )
        out = pl.pallas_call(
            kernel,
            out_shape=jax.ShapeDtypeStruct((NB, 2 * DM), BF16),
            in_specs=[pl.BlockSpec(memory_space=pl.ANY)] * len(args),
            scratch_shapes=[
                pltpu.VMEM((NB, DM), BF16),
                pltpu.VMEM((NB, DM), BF16),
                pltpu.VMEM((4, DM, 1024), BF16),
                pltpu.VMEM((4, 144, NH, DH), BF16),
                pltpu.VMEM((4, 128, NH, DH), BF16),
                pltpu.VMEM((4, 128, NH, DH), BF16),
                pltpu.VMEM((16, 1024, DC), BF16),
                pltpu.VMEM((nslot, 2, HG, run, DH), BF16),
                pltpu.VMEM((NO, DM, 512), BF16),
                pltpu.VMEM((NO, 4, DM, DH), BF16),
                pltpu.VMEM((NH, DM, DH), BF16),
                pltpu.VMEM((GPB, NB * HG, HG * DH), F32),
                pltpu.VMEM((NH, 8, DH), F32),
                pltpu.VMEM((4, NH * 8, 128), F32),
                pltpu.VMEM((4, NB * NH, 128), BF16),
                pltpu.VMEM((NB * NH, 128), F32),
                pltpu.VMEM((NB * NH, 128), F32),
                pltpu.VMEM((NB * NH, DC), F32),
                pltpu.VMEM((NO, 8, 512), F32),
                pltpu.VMEM((NH, 8, DH), F32),
                pltpu.SemaphoreType.DMA((7,)),
                pltpu.SemaphoreType.DMA((nslot,)),
                pltpu.SemaphoreType.DMA((NO,)),
            ],
            compiler_params=pltpu.CompilerParams(
                vmem_limit_bytes=100 * 1024 * 1024, disable_bounds_checks=nochk),
            name="fused_decode",
        )(*args)
        return out.reshape(NB, 1, 2 * DM)
    return f


@jax.jit
def pallas_concat_heads__mha_block_cached__compressed_kv_cla__decode_kernel(
    A_x, A_k_cache, A_v_cache, A_wq, A_wo, B_x, B_c_kv, B_w_q, B_w_uk, B_w_uv, B_w_o,
):
    return make()(A_x, A_k_cache, A_v_cache, A_wq, A_wo, B_x, B_c_kv, B_w_q, B_w_uk, B_w_uv, B_w_o)
```

```python
import functools

import jax
import jax.numpy as jnp
from jax import lax
import jax.experimental.pallas as pl
import jax.experimental.pallas.tpu as pltpu

BF16 = jnp.bfloat16
F32 = jnp.float32

NB, NH, SK, DH, DM, DC = 4, 32, 4096, 128, 576, 512
SCALE = DH ** -0.5

HG = 8
GPB = NH // HG
NG = NB * GPB
RUN = 256
SPG = SK // RUN
NKV = NG * SPG
NOUT = 8
AHEAD = 5
NSLOT = 8
assert AHEAD < NSLOT and AHEAD <= NOUT


def _nn(a, b):
    return jnp.dot(a, b, preferred_element_type=F32)


def _nt(a, b):
    return lax.dot_general(a, b, (((1,), (1,)), ((), ())), preferred_element_type=F32)


def _iota(shape, dim):
    return lax.broadcasted_iota(jnp.int32, shape, dim)


def _block(i, size):
    return pl.ds(pl.multiple_of(i * size, size), size)


def _loop(n, fn):
    def body(t, carry):
        fn(t)
        return carry
    lax.fori_loop(0, n, body, 0)


def _start(src, dst, sem, queue):
    pltpu.make_async_copy(src, dst, sem).start(priority=queue)


def _wait(buf, sem):
    pltpu.make_async_copy(buf, buf, sem).wait()


def _head_major_to_batch_major(transpose):
    shape = (8 * NH, NB * NH) if transpose else (NB * NH, 8 * NH)
    bh = _iota(shape, int(transpose))
    hb = _iota(shape, 1 - int(transpose))
    return jnp.where(hb == (bh % NH) * 8 + bh // NH, 1.0, 0.0).astype(BF16)


def _softmax_step(s, m_old):
    tiles = s.shape[1] // 128
    m_new = jnp.maximum(m_old, jnp.max(s, axis=1, keepdims=True))
    alpha = jnp.exp(m_old - m_new)
    p = jnp.exp(s - jnp.tile(m_new, (1, tiles)))
    lane_sums = p[:, :128]
    for t in range(1, tiles):
        lane_sums = lane_sums + p[:, t * 128:(t + 1) * 128]
    return p.astype(BF16), m_new, alpha, lane_sums


def _body(xa_h, k_h, v_h, wq_h, wo_h, xb_h, c_h, bq_h, uk_h, uv_h, bo_h, out_ref, *,
          xa_v, xb_v, wq_v, bq_v, uk_v, uv_v, c_v, kv_v, wo_v, bo_v,
          qa_v, oa_v, bqt_v, qb_v, ql_v, m_v, l_v, acc_v, lat_v, ob_v,
          sem_w, sem_kv, sem_wo, sem_bo):

    def issue_q_weights(t):
        def piece_a(p):
            rows = _block(p // 4, 8)
            _start(wq_h.at[rows, _block(p % 4, HG * DH)], wq_v.at[p % 4, rows], sem_w.at[0], 0)

        def piece_b(p):
            rows = pl.ds(2 * p, 2)
            _start(bq_h.at[rows], bq_v.at[rows], sem_w.at[1], 1)

        for s in range(2):
            for piece in (piece_a, piece_b):
                piece(s * 64 + t)
                piece((s + 2) * 64 + t)

        @pl.when(t < 32)
        def _():
            piece_a(256 + t)
            piece_b(256 + t)

    def issue_up_weights(t):
        for s in range(2):
            idx = (slice(None), s, pl.ds(2 * t, 2))
            _start(uk_h.at[idx], uk_v.at[idx], sem_w.at[2], 0)
            _start(uv_h.at[idx], uv_v.at[idx], sem_w.at[3], 1)

    def issue_latent(t):
        for s in range(4):
            for queue in range(2):
                idx = (2 * queue + s // 2, slice(None), s % 2, _block(t, 16))
                _start(c_h.at[idx], c_v.at[idx], sem_w.at[4], queue)

    def issue_kv(i):
        def one_round(d):
            rows = _block((i % SPG) * (RUN // 64) + d, 64)
            for s in range(4):
                for a, src in enumerate((k_h, v_h)):
                    _start(src.at[i // SPG, s // 2, :, s % 2, rows],
                           kv_v.at[i % NSLOT, a, s // 2, :, s % 2, _block(d, 64)],
                           sem_kv.at[i % NSLOT], a)
        _loop(RUN // 64, one_round)

    def issue_out_weights(i):
        def one_round(d):
            for s in range(2):
                rows = _block(s * 9 + d, 8)
                _start(wo_h.at[:, rows, _block(i, 4 * DH)], wo_v.at[i, :, rows], sem_wo.at[i], 0)
                pair, rows = pl.ds(2 * s, 2), _block(d, 64)
                _start(bo_h.at[pair, i, rows], bo_v.at[i, pair, rows], sem_bo.at[i], 1)
        _loop(9, one_round)

    _loop(64, issue_q_weights)
    _start(xa_h, xa_v, sem_w.at[5], 0)
    _start(xb_h, xb_v, sem_w.at[6], 1)
    _loop(64, issue_up_weights)
    _loop(64, issue_latent)
    _loop(AHEAD, issue_kv)
    for j, buf in enumerate((wq_v, bq_v, uk_v, uv_v, c_v, xa_v, xb_v)):
        _wait(buf, sem_w.at[j])

    m_v[...] = jnp.full(m_v.shape, -jnp.inf, F32)
    for ref in (l_v, acc_v, oa_v, ob_v):
        ref[...] = jnp.zeros(ref.shape, F32)

    def a_queries(c):
        x = xa_v[...].astype(F32)
        x = jnp.concatenate([jnp.broadcast_to(x[b:b + 1], (HG, DM)) for b in range(NB)], axis=0)
        q = _nn(x.astype(BF16), wq_v[c])
        qa_v[c] = jnp.where(_iota(q.shape, 0) % HG == _iota(q.shape, 1) // DH, q, 0.0)

    def b_split_heads(c):
        rows = pl.ds(pl.multiple_of(c * 48, 16), 48)
        bqt_v[:, rows, :] = jnp.swapaxes(bq_v[rows], 0, 1)

    def b_queries(c):
        x = xb_v[...].astype(F32)
        x = jnp.concatenate([x, jnp.zeros_like(x)], axis=0).astype(BF16)
        for j in range(4):
            qb_v[4 * c + j] = _nn(x, bqt_v[4 * c + j])

    def b_latent_queries(c):
        w = jnp.swapaxes(uk_v[c // 2, c % 2], 0, 1)
        q = jnp.concatenate([_nt(qb_v[h].astype(BF16), w[h]) for h in range(NH)], axis=0)
        ql_v[c] = _nn(_head_major_to_batch_major(False), q.astype(BF16)).astype(BF16)

    def b_attend(t):
        b = t // 8
        rows = _block(b, NH)
        c = c_v[b, (t // 4) % 2, (t // 2) % 2, _block(t % 2, 512)]
        q = jnp.concatenate([ql_v[j, rows] for j in range(DC // 128)], axis=1)
        p, m_new, alpha, lane_sums = _softmax_step(_nt(q, c) * SCALE, m_v[rows])
        m_v[rows] = m_new
        l_v[rows] = l_v[rows] * alpha + lane_sums
        acc_v[rows] = acc_v[rows] * jnp.tile(alpha, (1, DC // 128)) + _nn(p, c)

    def b_normalize(_):
        lat = acc_v[...] / jnp.sum(l_v[...], axis=1, keepdims=True)
        lat = _nn(_head_major_to_batch_major(True), lat.astype(BF16))
        for j in range(DC // 128):
            lat_v[j] = lat[:, j * 128:(j + 1) * 128]

    def b_context(c):
        w = jnp.swapaxes(uv_v[c // 2, c % 2], 0, 1)
        for h in range(NH):
            ob_v[h] += _nn(lat_v[c, pl.ds(8 * h, 8)].astype(BF16), w[h])

    jobs = ((a_queries, GPB), (b_split_heads, 12), (b_queries, 8), (b_latent_queries, 4),
            (b_attend, 32), (b_normalize, 1), (b_context, 4))
    assert 2 * sum(n for _, n in jobs) <= NKV

    def kv_step(i, carry):
        @pl.when(i % 2 == 0)
        def _():
            t, lo = i // 2, 0
            for job, n in jobs:
                pl.when((t >= lo) & (t < lo + n))(functools.partial(job, t - lo))
                lo += n

        pl.when(i + AHEAD < NKV)(functools.partial(issue_kv, i + AHEAD))
        pl.when(i + AHEAD >= NKV)(functools.partial(issue_out_weights, i + AHEAD - NKV))

        slot = i % NSLOT
        b, hg = (i // SPG) // GPB, (i // SPG) % GPB
        sublane = _iota((HG, DH), 0)
        first = i % SPG == 0
        m, l, acc = carry
        m = jnp.where(first, -jnp.inf, m)
        l = jnp.where(first, 0.0, l)
        acc = jnp.where(first, 0.0, acc)

        def head(a, j):
            return kv_v[slot, a, j // 4, (j // 2) % 2, j % 2]

        _wait(kv_v.at[slot], sem_kv.at[slot])
        q = qa_v[hg, _block(b, HG), :].astype(BF16)
        s = _nt(q[:, :DH], head(0, 0))
        for j in range(1, HG):
            s = s + _nt(q[:, j * DH:(j + 1) * DH], head(0, j))
        p, m, alpha, lane_sums = _softmax_step(s * SCALE, m)
        pv = _nn(p, head(1, 0))
        for j in range(1, HG):
            pv = jnp.where(sublane == j, _nn(p, head(1, j)), pv)
        l = l * alpha + lane_sums
        acc = acc * alpha + pv

        @pl.when(i % SPG == SPG - 1)
        def _():
            o = acc / jnp.sum(l, axis=1, keepdims=True)
            for j in range(HG):
                dst = (2 * hg + j // 4, slice(None), pl.ds((j % 4) * DH, DH))
                row = jnp.broadcast_to(o[j:j + 1], (HG, DH))
                oa_v[dst] = jnp.where(sublane == b, row, oa_v[dst])

        return m, l, acc

    zero = jnp.zeros((HG, DH), F32)
    lax.fori_loop(0, NKV, kv_step, (zero, zero, zero))

    lane_shift = DM % 128

    def out_step(i, carry):
        ya, yb = carry
        pl.when(i + AHEAD < NOUT)(functools.partial(issue_out_weights, i + AHEAD))
        _wait(wo_v.at[i], sem_wo.at[i])
        ya = ya + _nt(oa_v[i].astype(BF16), wo_v[i].reshape(DM, 4 * DH))
        _wait(bo_v.at[i], sem_bo.at[i])
        for j in range(4):
            w = jnp.concatenate([jnp.zeros((lane_shift, DH), BF16), bo_v[i, j]], axis=0)
            yb = yb + _nt(ob_v[NOUT * j + i].astype(BF16), w)
        return ya, yb

    ya, yb = lax.fori_loop(
        0, NOUT, out_step, (jnp.zeros((8, DM), F32), jnp.zeros((8, lane_shift + DM), F32)))
    out_ref[:, :DM] = ya[:NB].astype(BF16)
    out_ref[:, DM:] = yb[:NB, lane_shift:].astype(BF16)


def _kernel(*refs, **scratch):
    pl.run_scoped(
        functools.partial(_body, *refs, **scratch),
        sem_w=pltpu.SemaphoreType.DMA((7,)),
        sem_kv=pltpu.SemaphoreType.DMA((NSLOT,)),
        sem_wo=pltpu.SemaphoreType.DMA((NOUT,)),
        sem_bo=pltpu.SemaphoreType.DMA((NOUT,)),
    )


@jax.jit
def pallas_concat_heads__mha_block_cached__compressed_kv_cla__decode_kernel(
    A_x: jax.Array,
    A_k_cache: jax.Array,
    A_v_cache: jax.Array,
    A_wq: jax.Array,
    A_wo: jax.Array,
    B_x: jax.Array,
    B_c_kv: jax.Array,
    B_w_q: jax.Array,
    B_w_uk: jax.Array,
    B_w_uv: jax.Array,
    B_w_o: jax.Array,
):
    operands = (
        A_x.reshape(NB, DM),
        A_k_cache.reshape(NG, 2, 2, 2, SK, DH),
        A_v_cache.reshape(NG, 2, 2, 2, SK, DH),
        A_wq,
        A_wo.T.reshape(4, DM // 4, NH * DH),
        B_x.reshape(NB, DM),
        B_c_kv.reshape(NB, 2, 2, SK // 4, DC),
        B_w_q,
        B_w_uk.reshape(2, 2, DC // 4, NH, DH),
        B_w_uv.reshape(2, 2, DC // 4, NH, DH),
        B_w_o.transpose(0, 2, 1).reshape(4, NOUT, DM, DH),
    )
    out = pl.pallas_call(
        _kernel,
        out_shape=jax.ShapeDtypeStruct((NB, 2 * DM), BF16),
        in_specs=[pl.BlockSpec(memory_space=pl.ANY)] * len(operands),
        scratch_shapes=dict(
            xa_v=pltpu.VMEM((NB, DM), BF16),
            xb_v=pltpu.VMEM((NB, DM), BF16),
            wq_v=pltpu.VMEM((GPB, DM, HG * DH), BF16),
            bq_v=pltpu.VMEM((DM, NH, DH), BF16),
            uk_v=pltpu.VMEM((2, 2, DC // 4, NH, DH), BF16),
            uv_v=pltpu.VMEM((2, 2, DC // 4, NH, DH), BF16),
            c_v=pltpu.VMEM((NB, 2, 2, SK // 4, DC), BF16),
            kv_v=pltpu.VMEM((NSLOT, 2, 2, 2, 2, RUN, DH), BF16),
            wo_v=pltpu.VMEM((NOUT, 4, DM // 4, 4 * DH), BF16),
            bo_v=pltpu.VMEM((NOUT, 4, DM, DH), BF16),
            qa_v=pltpu.VMEM((GPB, NB * HG, HG * DH), F32),
            oa_v=pltpu.VMEM((NOUT, 8, 4 * DH), F32),
            bqt_v=pltpu.VMEM((NH, DM, DH), BF16),
            qb_v=pltpu.VMEM((NH, 8, DH), F32),
            ql_v=pltpu.VMEM((DC // 128, NB * NH, 128), BF16),
            m_v=pltpu.VMEM((NB * NH, 128), F32),
            l_v=pltpu.VMEM((NB * NH, 128), F32),
            acc_v=pltpu.VMEM((NB * NH, DC), F32),
            lat_v=pltpu.VMEM((DC // 128, 8 * NH, 128), F32),
            ob_v=pltpu.VMEM((NH, 8, DH), F32),
        ),
        compiler_params=pltpu.CompilerParams(vmem_limit_bytes=96 * 1024 * 1024),
        name="fused_decode",
    )(*operands)
    return out.reshape(NB, 1, 2 * DM)
```
